```python
import os as _os
_os.environ.setdefault("JAX_PLATFORMS", "cpu")
import jax
import jax.numpy as jnp

def _softmax(x, axis=-1):
    return jax.nn.softmax(x, axis=axis)
def _gelu(x):
    return jax.nn.gelu(x, approximate=True)
def _silu(x):
    return jax.nn.silu(x)
def _sigmoid(x):
    return jax.nn.sigmoid(x)
def _layernorm(x, axis=-1, eps=1e-5):
    m = jnp.mean(x, axis=axis, keepdims=True)
    v = jnp.var(x, axis=axis, keepdims=True)
    return (x - m) / jnp.sqrt(v + eps)
def _scatter_add(tgt, idx, src, axis=0):
    return tgt.at[idx].add(src)
def _segment_sum(src, seg, n):
    return jax.ops.segment_sum(src, seg, n)
class _Rng:
    def __init__(self, key):
        self._k = key
    def _next(self):
        self._k, sub = jax.random.split(self._k)
        return sub
    def normal(self, shape):
        return jax.random.normal(self._next(), shape, dtype=jnp.bfloat16)
    def randint(self, lo, hi, shape):
        return jax.random.randint(self._next(), shape, lo, hi, dtype=jnp.int32)
    def uniform(self, shape, lo=0.0, hi=1.0):
        return jax.random.uniform(self._next(), shape, jnp.bfloat16, lo, hi)
    def permutation(self, n):
        return jax.random.permutation(self._next(), n)


kernel_name = 'parallel_sum__ssm_conv_s5__geglu_ffn__prompt'

def setup_inputs():
    _rng = _Rng(jax.random.key(int.from_bytes(__import__("os").urandom(4), "little")))
    _w = (lambda a: (lambda t: t.astype(jnp.bfloat16) if jnp.issubdtype(t.dtype, jnp.floating) else t)(jnp.asarray(a)))
    def _A_setup():
        B, S, D = 1, 2048, 512
        P = D
        Lambda_re = -0.5 * jnp.exp((lambda *s: _rng.normal(s) * 0.8)(P))
        Lambda_im = (lambda *s: _rng.normal(s) * 0.8)(P) * 1.0
        B_re = (lambda *s: _rng.normal(s) * 0.8)(P, D) * (D ** -0.5)
        B_im = (lambda *s: _rng.normal(s) * 0.8)(P, D) * (D ** -0.5)
        C_re = (lambda *s: _rng.normal(s) * 0.8)(D, P) * (P ** -0.5)
        C_im = (lambda *s: _rng.normal(s) * 0.8)(D, P) * (P ** -0.5)
        log_dt = (lambda *s: _rng.normal(s) * 0.8)(P) * 0.3 - 2.0
        Dskip = (lambda *s: _rng.normal(s) * 0.8)(D)
        return {
            "x": _w((lambda *s: _rng.normal(s) * 0.05)(B, S, D)),
            "Lambda_re": _w(Lambda_re),
            "Lambda_im": _w(Lambda_im),
            "B_re": _w(B_re),
            "B_im": _w(B_im),
            "C_re": _w(C_re),
            "C_im": _w(C_im),
            "log_dt": _w(log_dt),
            "Dskip": _w(Dskip),
        }
    _A_in = _A_setup()

    def _B_setup():
        B, S, D, F = 1, 2048, 512, 1376
        return {
            "x": _w((lambda *s: _rng.normal(s) * 0.05)(B, S, D)),
            "w_gate": _w((lambda *s: _rng.normal(s) * 0.05)(D, F)),
            "w_up": _w((lambda *s: _rng.normal(s) * 0.05)(D, F)),
            "w_down": _w((lambda *s: _rng.normal(s) * 0.05)(F, D)),
        }
    _B_in = _B_setup()

    return {
        "A_x": _A_in["x"],
        "A_Lambda_re": _A_in["Lambda_re"],
        "A_Lambda_im": _A_in["Lambda_im"],
        "A_B_re": _A_in["B_re"],
        "A_B_im": _A_in["B_im"],
        "A_C_re": _A_in["C_re"],
        "A_C_im": _A_in["C_im"],
        "A_log_dt": _A_in["log_dt"],
        "A_Dskip": _A_in["Dskip"],
        "B_x": _B_in["x"],
        "B_w_gate": _B_in["w_gate"],
        "B_w_up": _B_in["w_up"],
        "B_w_down": _B_in["w_down"],
    }

def reference(A_x, A_Lambda_re, A_Lambda_im, A_B_re, A_B_im, A_C_re, A_C_im, A_log_dt, A_Dskip, B_x, B_w_gate, B_w_up, B_w_down):
    def _A_ref(x, Lambda_re, Lambda_im, B_re, B_im, C_re, C_im, log_dt, Dskip):
        Bsz, L, H = x.shape
        Lam = Lambda_re + 1j * Lambda_im
        Bmat = B_re + 1j * B_im
        Cmat = C_re + 1j * C_im
        dt = jnp.exp(log_dt)
        Lam_bar = jnp.exp(dt * Lam)
        B_bar = ((Lam_bar - 1.0) / Lam)[:, None] * Bmat
        Bu = jnp.einsum("bld,pd->blp", x + 0j, B_bar)
        h = jnp.zeros_like(Bu[:, 0, :])
        hs = []
        for t in range(L):
            h = Lam_bar[None, :] * h + Bu[:, t, :]
            hs.append(h)
        hseq = jnp.stack(hs, 1)
        y = 2.0 * jnp.einsum("blp,dp->bld", hseq, Cmat).real + x * Dskip[None, None, :]
        return y

    def _B_ref(x, w_gate, w_up, w_down):
        return (_gelu(x @ w_gate) * (x @ w_up)) @ w_down

    x = A_x
    xn = _layernorm(x, axis=-1)
    return x + _A_ref(xn, A_Lambda_re, A_Lambda_im, A_B_re, A_B_im, A_C_re, A_C_im, A_log_dt, A_Dskip) + _B_ref(xn, B_w_gate, B_w_up, B_w_down)
```

```python
import functools
import jax
import jax.numpy as jnp
from jax import lax
import jax.experimental.pallas as pl
import jax.experimental.pallas.tpu as pltpu

L, D, P, F = 2048, 512, 512, 1376
LC = 512
NC = L // LC
S = 8
T = LC // S
TP = T + 1
HC = LC // 2
NOB = 4

_NT = (((1,), (1,)), ((), ()))


def _cmul(ar, ai, br, bi):
    return ar * br - ai * bi, ar * bi + ai * br


def _kernel(lre_r, lim_r, ldt_r, dsk_ref,
            x_hbm, bre_hbm, bim_hbm, cre_hbm, cim_hbm, wg_hbm, wu_hbm, wd_hbm,
            o_hbm,
            x_ref, bre_ref, bim_ref, cre_ref, cim_ref, wg_ref, wu_ref, wd_ref, sems, xsems,
            ccat_ref, a_ref, carry_ref, bu_ref, h_ref, xnb_ref, base_ref, obuf, osems):
    step = pl.program_id(0)
    slot = step % 2

    srcs = (bre_hbm, bim_hbm, wg_hbm, wu_hbm, cre_hbm, cim_hbm, wd_hbm)
    dsts = (bre_ref, bim_ref, wg_ref, wu_ref, cre_ref, cim_ref, wd_ref)

    def rows(c, n):
        return pl.ds(c * n if isinstance(c, int) else pl.multiple_of(c * n, n), n)

    def cp(i):
        return pltpu.make_async_copy(srcs[i], dsts[i], sems.at[i])

    def cpx(c):
        return pltpu.make_async_copy(x_hbm.at[rows(c, HC)], x_ref.at[rows(c, HC)], xsems.at[c])

    def cpo(hc):
        b = hc % NOB
        return pltpu.make_async_copy(obuf.at[b], o_hbm.at[rows(hc, HC)], osems.at[b])

    def row(r):
        return r[...].reshape(1, P).astype(jnp.float32)

    def layernorm(xb):
        x = xb.astype(jnp.float32)
        m = jnp.mean(x, axis=-1, keepdims=True)
        xc = x - m
        v = jnp.mean(xc * xc, axis=-1, keepdims=True)
        xn = xc * lax.rsqrt(v + 1e-5)
        return xn.astype(jnp.bfloat16), x + xn * a_ref[4:5, :]

    def store_bu(val, jo, s0):
        for j in range(4):
            for s in range(val.shape[0] // T):
                bu_ref[jo + j, pl.ds(TP * (s0 + s), T), :] = val[T * s:T * (s + 1), j * 128:(j + 1) * 128]

    def scan():
        def ld(t, lo):
            return jnp.concatenate([bu_ref[j, pl.ds(t, S, stride=TP), :] for j in range(lo, lo + 4)], axis=1)

        ar = jnp.broadcast_to(a_ref[0:1, :], (S, P))
        ai = jnp.broadcast_to(a_ref[1:2, :], (S, P))

        hr = jnp.zeros((S, P), jnp.float32)
        hi = jnp.zeros((S, P), jnp.float32)
        for t in range(T):
            ur = ld(t, 0)
            ui = ld(t, 4)
            hr, hi = ar * hr - ai * hi + ur, ar * hi + ai * hr + ui

        atr = a_ref[2:3, :]
        ati = a_ref[3:4, :]
        cr = carry_ref[0:1, :]
        ci = carry_ref[1:2, :]
        rows_r = []
        rows_i = []
        for s in range(S):
            rows_r.append(cr)
            rows_i.append(ci)
            er = hr[s:s + 1, :]
            ei = hi[s:s + 1, :]
            cr, ci = atr * cr - ati * ci + er, atr * ci + ati * cr + ei
        carry_ref[0:1, :] = cr
        carry_ref[1:2, :] = ci
        hr = jnp.concatenate(rows_r, axis=0)
        hi = jnp.concatenate(rows_i, axis=0)

        for t in range(T):
            ur = ld(t, 0)
            ui = ld(t, 4)
            hr, hi = ar * hr - ai * hi + ur, ar * hi + ai * hr + ui
            for j in range(4):
                h_ref[j, pl.ds(t, S, stride=TP), :] = hr[:, j * 128:(j + 1) * 128]
                h_ref[4 + j, pl.ds(t, S, stride=TP), :] = hi[:, j * 128:(j + 1) * 128]

    def ln_next(nxt, nslot):
        xnb_n, base_n = layernorm(x_ref[rows(nxt, LC), :])
        xnb_ref[...] = xnb_n
        base_ref[nslot] = base_n

    def finish(act, base_fn, hc0):
        for hh in range(2):
            s0 = hh * (S // 2)
            hcat = jnp.concatenate(
                [jnp.concatenate([h_ref[j, pl.ds(TP * s, T), :] for s in range(s0, s0 + S // 2)], axis=0)
                 for j in range(8)], axis=1).astype(jnp.bfloat16)
            y = lax.dot_general(hcat, ccat_ref[...], _NT, preferred_element_type=jnp.float32)
            dn = jnp.dot(act[hh * HC:(hh + 1) * HC], wd_ref[...], preferred_element_type=jnp.float32)
            hc = hc0 + hh
            obuf[hc % NOB] = base_fn(hh) + y + dn
            cpo(hc).start()

    @pl.when(step == 0)
    def _first():
        cpx(0).start()
        cp(0).start()
        cpx(1).start()
        cp(1).start()
        lre = row(lre_r)
        lim = row(lim_r)
        dt = jnp.exp(row(ldt_r)).astype(jnp.bfloat16).astype(jnp.float32)
        mag = jnp.exp(dt * lre)
        ar = mag * jnp.cos(dt * lim)
        ai = mag * jnp.sin(dt * lim)
        nr = ar - 1.0
        ni = ai
        den = lre * lre + lim * lim
        cfr = (nr * lre + ni * lim) / den
        cfi = (ni * lre - nr * lim) / den
        a_ref[0:1, :] = ar
        a_ref[1:2, :] = ai
        pr, pi = ar, ai
        k = 1
        while k < T:
            pr, pi = _cmul(pr, pi, pr, pi)
            k *= 2
        a_ref[2:3, :] = pr
        a_ref[3:4, :] = pi
        a_ref[4:5, :] = row(dsk_ref)
        a_ref[5:8, :] = jnp.zeros((3, P), jnp.float32)
        carry_ref[...] = jnp.zeros((8, P), jnp.float32)

        cpx(0).wait()
        xa, base_a = layernorm(x_ref[0:HC, :])
        cp(0).wait()
        cpx(1).wait()
        cp(2).start()
        store_bu(lax.dot_general(xa, bre_ref[...], _NT, preferred_element_type=jnp.float32), 0, 0)
        xb, base_b = layernorm(x_ref[HC:LC, :])
        store_bu(lax.dot_general(xb, bre_ref[...], _NT, preferred_element_type=jnp.float32), 0, S // 2)
        xnb = jnp.concatenate([xa, xb], axis=0)
        cp(1).wait()
        store_bu(lax.dot_general(xnb, bim_ref[...], _NT, preferred_element_type=jnp.float32), 4, 0)
        cp(2).wait()
        cp(3).start()
        cp(4).start()
        cp(5).start()
        g = lax.dot_general(xnb, wg_ref[...], _NT, preferred_element_type=jnp.float32)
        scan()
        cp(3).wait()
        cp(6).start()
        for c in range(2, 2 * NC):
            cpx(c).start()
        u = lax.dot_general(xnb, wu_ref[...], _NT, preferred_element_type=jnp.float32)
        act = (jax.nn.gelu(g, approximate=True) * u).astype(jnp.bfloat16)
        cpx(2).wait()
        cpx(3).wait()
        cp(4).wait()
        cp(5).wait()
        cp(6).wait()
        ln_next(1, 1)
        c_re = cre_ref[...].astype(jnp.float32)
        c_im = cim_ref[...].astype(jnp.float32)
        ccat_ref[:, 0:P] = (2.0 * (c_re * cfr - c_im * cfi)).astype(jnp.bfloat16)
        ccat_ref[:, P:2 * P] = (-2.0 * (c_re * cfi + c_im * cfr)).astype(jnp.bfloat16)
        finish(act, lambda hh: (base_a, base_b)[hh], 0)

    @pl.when(step > 0)
    def _rest():
        @pl.when(step < NC - 1)
        def _():
            cpx(2 * step + 2).wait()
            cpx(2 * step + 3).wait()

        @pl.when(step >= NOB // 2)
        def _():
            cpo(2 * step - NOB).wait()
            cpo(2 * step + 1 - NOB).wait()

        xnb = xnb_ref[...]
        store_bu(lax.dot_general(xnb, bre_ref[...], _NT, preferred_element_type=jnp.float32), 0, 0)
        store_bu(lax.dot_general(xnb, bim_ref[...], _NT, preferred_element_type=jnp.float32), 4, 0)
        g = lax.dot_general(xnb, wg_ref[...], _NT, preferred_element_type=jnp.float32)
        u = lax.dot_general(xnb, wu_ref[...], _NT, preferred_element_type=jnp.float32)
        act = (jax.nn.gelu(g, approximate=True) * u).astype(jnp.bfloat16)
        scan()
        ln_next(jnp.minimum(step + 1, NC - 1), 1 - slot)
        finish(act, lambda hh: base_ref[slot, hh * HC:(hh + 1) * HC, :], 2 * step)

        @pl.when(step == NC - 1)
        def _():
            for hc in range(2 * NC - NOB, 2 * NC):
                cpo(hc).wait()


@jax.jit
def pallas_parallel_sum__ssm_conv_s5__geglu_ffn__prompt_kernel(
    A_x, A_Lambda_re, A_Lambda_im, A_B_re, A_B_im, A_C_re, A_C_im, A_log_dt, A_Dskip,
    B_x, B_w_gate, B_w_up, B_w_down,
):
    x2 = A_x.reshape(L, D)
    full = lambda shape: pl.BlockSpec(shape, lambda i: (0,) * len(shape))
    anyspec = pl.BlockSpec(memory_space=pl.ANY)
    out = pl.pallas_call(
        _kernel,
        grid=(NC,),
        in_specs=[
            full((P,)), full((P,)), full((P,)),
            full((D,)),
            anyspec, anyspec, anyspec, anyspec, anyspec, anyspec, anyspec, anyspec,
        ],
        out_specs=anyspec,
        out_shape=jax.ShapeDtypeStruct((L, D), jnp.float32),
        scratch_shapes=[
            pltpu.VMEM((L, D), jnp.bfloat16),
            pltpu.VMEM((P, D), jnp.bfloat16),
            pltpu.VMEM((P, D), jnp.bfloat16),
            pltpu.VMEM((D, P), jnp.bfloat16),
            pltpu.VMEM((D, P), jnp.bfloat16),
            pltpu.VMEM((F, D), jnp.bfloat16),
            pltpu.VMEM((F, D), jnp.bfloat16),
            pltpu.VMEM((F, D), jnp.bfloat16),
            pltpu.SemaphoreType.DMA((7,)),
            pltpu.SemaphoreType.DMA((2 * NC,)),
            pltpu.VMEM((D, 2 * P), jnp.bfloat16),
            pltpu.VMEM((8, P), jnp.float32),
            pltpu.VMEM((8, P), jnp.float32),
            pltpu.VMEM((8, S * TP, 128), jnp.float32),
            pltpu.VMEM((8, S * TP, 128), jnp.float32),
            pltpu.VMEM((LC, D), jnp.bfloat16),
            pltpu.VMEM((2, LC, D), jnp.float32),
            pltpu.VMEM((NOB, HC, D), jnp.float32),
            pltpu.SemaphoreType.DMA((NOB,)),
        ],
        compiler_params=pltpu.CompilerParams(
            dimension_semantics=("arbitrary",),
            vmem_limit_bytes=64 * 1024 * 1024,
        ),
    )(A_Lambda_re, A_Lambda_im, A_log_dt, A_Dskip,
      x2, A_B_re, A_B_im, A_C_re, A_C_im, B_w_gate.T, B_w_up.T, B_w_down)
    return out.reshape(1, L, D)
```

```python
import jax
import jax.numpy as jnp
from jax import lax
import jax.experimental.pallas as pl
import jax.experimental.pallas.tpu as pltpu

L, D, P, F = 2048, 512, 512, 1376
LC = 512
NC = L // LC
S = 8
T = LC // S
TP = T + 1
HC = LC // 2
PIECES = ((0, 256), (256, 128), (384, 128))
NP = len(PIECES)

_NT = (((1,), (1,)), ((), ()))


def _cmul(ar, ai, br, bi):
    return ar * br - ai * bi, ar * bi + ai * br


def _kernel(lre_r, lim_r, ldt_r, dsk_ref,
            x_hbm, bre_hbm, bim_hbm, cre_hbm, cim_hbm, wg_hbm, wu_hbm, wd_hbm,
            o_hbm,
            x_ref, bre_ref, bim_ref, cre_ref, cim_ref, wg_ref, wu_ref, wd_ref, sems, xsems,
            ccat_ref, a_ref, carry_ref, bu_ref, h_ref, st_ref, obuf, osems):
    step = pl.program_id(0)
    slot = step % 2

    srcs = (bre_hbm, bim_hbm, wg_hbm, wu_hbm, cre_hbm, cim_hbm, wd_hbm)
    dsts = (bre_ref, bim_ref, wg_ref, wu_ref, cre_ref, cim_ref, wd_ref)

    def rows(c, n):
        return pl.ds(c * n if isinstance(c, int) else pl.multiple_of(c * n, n), n)

    def cp(i):
        return pltpu.make_async_copy(srcs[i], dsts[i], sems.at[i])

    def cpx(c):
        return pltpu.make_async_copy(x_hbm.at[rows(c, HC)], x_ref.at[rows(c, HC)], xsems.at[c])

    def cpo(c, k):
        off, n = PIECES[k]
        start = c * LC + off if isinstance(c, int) else pl.multiple_of(c * LC + off, 128)
        return pltpu.make_async_copy(obuf.at[c, pl.ds(off, n)], o_hbm.at[pl.ds(start, n)],
                                     osems.at[c * NP + k])

    def row(r):
        return r[...].reshape(1, P).astype(jnp.float32)

    def stats(xb):
        x = xb.astype(jnp.float32)
        m = jnp.mean(x, axis=-1, keepdims=True)
        xc = x - m
        v = jnp.mean(xc * xc, axis=-1, keepdims=True)
        return m, lax.rsqrt(v + 1e-5)

    def normalize(xb, m, r):
        x = xb.astype(jnp.float32)
        m4 = jnp.concatenate([m] * (D // 128), axis=1)
        r4 = jnp.concatenate([r] * (D // 128), axis=1)
        return x, (x - m4) * r4

    def bcast(v):
        return jnp.broadcast_to(v, (v.shape[0], 128))

    def store_bu(val, jo, s0):
        for j in range(4):
            for s in range(val.shape[0] // T):
                bu_ref[jo + j, pl.ds(TP * (s0 + s), T), :] = val[T * s:T * (s + 1), j * 128:(j + 1) * 128]

    def scan():
        def ld(t, lo):
            return jnp.concatenate([bu_ref[j, pl.ds(t, S, stride=TP), :] for j in range(lo, lo + 4)], axis=1)

        ar = jnp.broadcast_to(a_ref[0:1, :], (S, P))
        ai = jnp.broadcast_to(a_ref[1:2, :], (S, P))

        hr = jnp.zeros((S, P), jnp.float32)
        hi = jnp.zeros((S, P), jnp.float32)
        for t in range(T):
            ur = ld(t, 0)
            ui = ld(t, 4)
            hr, hi = ar * hr - ai * hi + ur, ar * hi + ai * hr + ui

        atr = a_ref[2:3, :]
        ati = a_ref[3:4, :]
        cr = carry_ref[0:1, :]
        ci = carry_ref[1:2, :]
        rows_r = []
        rows_i = []
        for s in range(S):
            rows_r.append(cr)
            rows_i.append(ci)
            er = hr[s:s + 1, :]
            ei = hi[s:s + 1, :]
            cr, ci = atr * cr - ati * ci + er, atr * ci + ati * cr + ei
        carry_ref[0:1, :] = cr
        carry_ref[1:2, :] = ci
        hr = jnp.concatenate(rows_r, axis=0)
        hi = jnp.concatenate(rows_i, axis=0)

        for t in range(T):
            ur = ld(t, 0)
            ui = ld(t, 4)
            hr, hi = ar * hr - ai * hi + ur, ar * hi + ai * hr + ui
            for j in range(4):
                h_ref[j, pl.ds(t, S, stride=TP), :] = hr[:, j * 128:(j + 1) * 128]
                h_ref[4 + j, pl.ds(t, S, stride=TP), :] = hi[:, j * 128:(j + 1) * 128]

    def ln_next(nxt, nslot):
        m, r = stats(x_ref[rows(nxt, LC), :])
        st_ref[nslot, 0] = bcast(m)
        st_ref[nslot, 1] = bcast(r)

    def finish(act, c, sl):
        for k, (off, n) in enumerate(PIECES):
            parts = []
            for j in range(8):
                segs = []
                for s in range(off // T, (off + n) // T):
                    segs.append(h_ref[j, pl.ds(TP * s, T), :])
                parts.append(jnp.concatenate(segs, axis=0))
            hcat = jnp.concatenate(parts, axis=1).astype(jnp.bfloat16)
            y = lax.dot_general(hcat, ccat_ref[...], _NT, preferred_element_type=jnp.float32)
            dn = jnp.dot(act[off:off + n], wd_ref[...], preferred_element_type=jnp.float32)
            start = c * LC + off if isinstance(c, int) else pl.multiple_of(c * LC + off, 128)
            x, xn = normalize(x_ref[pl.ds(start, n), :], st_ref[sl, 0, off:off + n, :],
                              st_ref[sl, 1, off:off + n, :])
            obuf[c, off:off + n, :] = (x + xn * a_ref[4:5, :]) + y + dn
            cpo(c, k).start()

    @pl.when(step == 0)
    def _first():
        cpx(0).start()
        cp(0).start()
        cpx(1).start()
        cp(1).start()
        lre = row(lre_r)
        lim = row(lim_r)
        dt = jnp.exp(row(ldt_r)).astype(jnp.bfloat16).astype(jnp.float32)
        mag = jnp.exp(dt * lre)
        ar = mag * jnp.cos(dt * lim)
        ai = mag * jnp.sin(dt * lim)
        nr = ar - 1.0
        ni = ai
        den = lre * lre + lim * lim
        cfr = (nr * lre + ni * lim) / den
        cfi = (ni * lre - nr * lim) / den
        a_ref[0:1, :] = ar
        a_ref[1:2, :] = ai
        pr, pi = ar, ai
        k = 1
        while k < T:
            pr, pi = _cmul(pr, pi, pr, pi)
            k *= 2
        a_ref[2:3, :] = pr
        a_ref[3:4, :] = pi
        a_ref[4:5, :] = row(dsk_ref)
        a_ref[5:8, :] = jnp.zeros((3, P), jnp.float32)
        carry_ref[...] = jnp.zeros((8, P), jnp.float32)

        cpx(0).wait()
        ma, ra = stats(x_ref[0:HC, :])
        ma, ra = bcast(ma), bcast(ra)
        st_ref[0, 0, 0:HC, :] = ma
        st_ref[0, 1, 0:HC, :] = ra
        xa = normalize(x_ref[0:HC, :], ma, ra)[1].astype(jnp.bfloat16)
        cp(0).wait()
        cpx(1).wait()
        cp(2).start()
        store_bu(lax.dot_general(xa, bre_ref[...], _NT, preferred_element_type=jnp.float32), 0, 0)
        mb, rb = stats(x_ref[HC:LC, :])
        mb, rb = bcast(mb), bcast(rb)
        st_ref[0, 0, HC:LC, :] = mb
        st_ref[0, 1, HC:LC, :] = rb
        xb = normalize(x_ref[HC:LC, :], mb, rb)[1].astype(jnp.bfloat16)
        store_bu(lax.dot_general(xb, bre_ref[...], _NT, preferred_element_type=jnp.float32), 0, S // 2)
        xnb = jnp.concatenate([xa, xb], axis=0)
        cp(1).wait()
        store_bu(lax.dot_general(xnb, bim_ref[...], _NT, preferred_element_type=jnp.float32), 4, 0)
        cp(2).wait()
        cp(3).start()
        cp(4).start()
        cp(5).start()
        g = lax.dot_general(xnb, wg_ref[...], _NT, preferred_element_type=jnp.float32)
        scan()
        cp(3).wait()
        cp(6).start()
        for c in range(2, 2 * NC):
            cpx(c).start()
        u = lax.dot_general(xnb, wu_ref[...], _NT, preferred_element_type=jnp.float32)
        act = (jax.nn.gelu(g, approximate=True) * u).astype(jnp.bfloat16)
        cpx(2).wait()
        cpx(3).wait()
        cp(4).wait()
        cp(5).wait()
        cp(6).wait()
        ln_next(1, 1)
        c_re = cre_ref[...].astype(jnp.float32)
        c_im = cim_ref[...].astype(jnp.float32)
        ccat_ref[:, 0:P] = (2.0 * (c_re * cfr - c_im * cfi)).astype(jnp.bfloat16)
        ccat_ref[:, P:2 * P] = (-2.0 * (c_re * cfi + c_im * cfr)).astype(jnp.bfloat16)
        finish(act, 0, 0)
        for c in range(4, 2 * NC):
            cpx(c).wait()

    @pl.when(step > 0)
    def _rest():
        xnb = normalize(x_ref[rows(step, LC), :], st_ref[slot, 0], st_ref[slot, 1])[1].astype(jnp.bfloat16)
        store_bu(lax.dot_general(xnb, bre_ref[...], _NT, preferred_element_type=jnp.float32), 0, 0)
        store_bu(lax.dot_general(xnb, bim_ref[...], _NT, preferred_element_type=jnp.float32), 4, 0)
        g = lax.dot_general(xnb, wg_ref[...], _NT, preferred_element_type=jnp.float32)
        u = lax.dot_general(xnb, wu_ref[...], _NT, preferred_element_type=jnp.float32)
        act = (jax.nn.gelu(g, approximate=True) * u).astype(jnp.bfloat16)
        scan()
        ln_next(jnp.minimum(step + 1, NC - 1), 1 - slot)
        finish(act, step, slot)

        @pl.when(step == NC - 1)
        def _():
            for c in range(NC):
                for k in range(NP):
                    cpo(c, k).wait()


@jax.jit
def pallas_parallel_sum__ssm_conv_s5__geglu_ffn__prompt_kernel(
    A_x, A_Lambda_re, A_Lambda_im, A_B_re, A_B_im, A_C_re, A_C_im, A_log_dt, A_Dskip,
    B_x, B_w_gate, B_w_up, B_w_down,
):
    x2 = A_x.reshape(L, D)
    full = lambda shape: pl.BlockSpec(shape, lambda i: (0,) * len(shape))
    anyspec = pl.BlockSpec(memory_space=pl.ANY)
    out = pl.pallas_call(
        _kernel,
        grid=(NC,),
        in_specs=[
            full((P,)), full((P,)), full((P,)),
            full((D,)),
            anyspec, anyspec, anyspec, anyspec, anyspec, anyspec, anyspec, anyspec,
        ],
        out_specs=anyspec,
        out_shape=jax.ShapeDtypeStruct((L, D), jnp.float32),
        scratch_shapes=[
            pltpu.VMEM((L, D), jnp.bfloat16),
            pltpu.VMEM((P, D), jnp.bfloat16),
            pltpu.VMEM((P, D), jnp.bfloat16),
            pltpu.VMEM((D, P), jnp.bfloat16),
            pltpu.VMEM((D, P), jnp.bfloat16),
            pltpu.VMEM((F, D), jnp.bfloat16),
            pltpu.VMEM((F, D), jnp.bfloat16),
            pltpu.VMEM((F, D), jnp.bfloat16),
            pltpu.SemaphoreType.DMA((7,)),
            pltpu.SemaphoreType.DMA((2 * NC,)),
            pltpu.VMEM((D, 2 * P), jnp.bfloat16),
            pltpu.VMEM((8, P), jnp.float32),
            pltpu.VMEM((8, P), jnp.float32),
            pltpu.VMEM((8, S * TP, 128), jnp.float32),
            pltpu.VMEM((8, S * TP, 128), jnp.float32),
            pltpu.VMEM((2, 2, LC, 128), jnp.float32),
            pltpu.VMEM((NC, LC, D), jnp.float32),
            pltpu.SemaphoreType.DMA((NC * NP,)),
        ],
        compiler_params=pltpu.CompilerParams(
            dimension_semantics=("arbitrary",),
            vmem_limit_bytes=64 * 1024 * 1024,
        ),
    )(A_Lambda_re, A_Lambda_im, A_log_dt, A_Dskip,
      x2, A_B_re, A_B_im, A_C_re, A_C_im, B_w_gate.T, B_w_up.T, B_w_down)
    return out.reshape(1, L, D)
```

```python
import jax
import jax.numpy as jnp
from jax import lax
import jax.experimental.pallas as pl
import jax.experimental.pallas.tpu as pltpu

L, D, P, F = 2048, 512, 512, 1376
LC = 512
NC = L // LC
S = 8
T = LC // S
TP = T + 1
HC = LC // 2
PIECES = ((0, 256), (256, 128), (384, 128))
NP = len(PIECES)

_NT = (((1,), (1,)), ((), ()))


def _cmul(ar, ai, br, bi):
    return ar * br - ai * bi, ar * bi + ai * br


def _kernel(lre_r, lim_r, ldt_r, dsk_ref,
            x_hbm, bre_hbm, bim_hbm, cre_hbm, cim_hbm, wg_hbm, wu_hbm, wd_hbm,
            o_hbm,
            x_ref, bre_ref, bim_ref, cre_ref, cim_ref, wg_ref, wu_ref, wd_ref, sems, xsems,
            ccat_ref, a_ref, carry_ref, bu_ref, h_ref, st_ref, obuf, osems):
    step = pl.program_id(0)
    slot = step % 2

    srcs = (bre_hbm, bim_hbm, wg_hbm, wu_hbm, cre_hbm, cim_hbm, wd_hbm)
    dsts = (bre_ref, bim_ref, wg_ref, wu_ref, cre_ref, cim_ref, wd_ref)

    def rows(c, n):
        return pl.ds(c * n if isinstance(c, int) else pl.multiple_of(c * n, n), n)

    def cp(i):
        return pltpu.make_async_copy(srcs[i], dsts[i], sems.at[i])

    def cpx(c):
        return pltpu.make_async_copy(x_hbm.at[rows(c, HC)], x_ref.at[rows(c, HC)], xsems.at[c])

    def cpo(c, k):
        off, n = PIECES[k]
        start = c * LC + off if isinstance(c, int) else pl.multiple_of(c * LC + off, 128)
        return pltpu.make_async_copy(obuf.at[c, pl.ds(off, n)], o_hbm.at[pl.ds(start, n)],
                                     osems.at[c * NP + k])

    def row(r):
        return r[...].reshape(1, P).astype(jnp.float32)

    def stats(xb):
        x = xb.astype(jnp.float32)
        m = jnp.mean(x, axis=-1, keepdims=True)
        xc = x - m
        v = jnp.mean(xc * xc, axis=-1, keepdims=True)
        return m, lax.rsqrt(v + 1e-5)

    def normalize(xb, m, r):
        x = xb.astype(jnp.float32)
        m4 = jnp.concatenate([m] * (D // 128), axis=1)
        r4 = jnp.concatenate([r] * (D // 128), axis=1)
        return x, (x - m4) * r4

    def bcast(v):
        return jnp.broadcast_to(v, (v.shape[0], 128))

    def store_bu(val, jo, s0):
        for j in range(4):
            for s in range(val.shape[0] // T):
                bu_ref[jo + j, pl.ds(TP * (s0 + s), T), :] = val[T * s:T * (s + 1), j * 128:(j + 1) * 128]

    def scan(j0=0, nj=4):
        lo, hi_ = j0 * 128, (j0 + nj) * 128
        W = nj * 128

        def ld(t, base):
            return jnp.concatenate([bu_ref[base + j, pl.ds(t, S, stride=TP), :] for j in range(j0, j0 + nj)], axis=1)

        ar = jnp.broadcast_to(a_ref[0:1, lo:hi_], (S, W))
        ai = jnp.broadcast_to(a_ref[1:2, lo:hi_], (S, W))

        hr = jnp.zeros((S, W), jnp.float32)
        hi = jnp.zeros((S, W), jnp.float32)
        for t in range(T):
            ur = ld(t, 0)
            ui = ld(t, 4)
            hr, hi = ar * hr - ai * hi + ur, ar * hi + ai * hr + ui

        atr = a_ref[2:3, lo:hi_]
        ati = a_ref[3:4, lo:hi_]
        cr = carry_ref[0:1, lo:hi_]
        ci = carry_ref[1:2, lo:hi_]
        rows_r = []
        rows_i = []
        for s in range(S):
            rows_r.append(cr)
            rows_i.append(ci)
            er = hr[s:s + 1, :]
            ei = hi[s:s + 1, :]
            cr, ci = atr * cr - ati * ci + er, atr * ci + ati * cr + ei
        carry_ref[0:1, lo:hi_] = cr
        carry_ref[1:2, lo:hi_] = ci
        hr = jnp.concatenate(rows_r, axis=0)
        hi = jnp.concatenate(rows_i, axis=0)

        for t in range(T):
            ur = ld(t, 0)
            ui = ld(t, 4)
            hr, hi = ar * hr - ai * hi + ur, ar * hi + ai * hr + ui
            for j in range(nj):
                h_ref[j0 + j, pl.ds(t, S, stride=TP), :] = hr[:, j * 128:(j + 1) * 128]
                h_ref[4 + j0 + j, pl.ds(t, S, stride=TP), :] = hi[:, j * 128:(j + 1) * 128]

    def ln_next(nxt, nslot):
        m, r = stats(x_ref[rows(nxt, LC), :])
        st_ref[nslot, 0] = bcast(m)
        st_ref[nslot, 1] = bcast(r)

    def finish(act, c, sl):
        for k, (off, n) in enumerate(PIECES):
            parts = []
            for j in range(8):
                segs = []
                for s in range(off // T, (off + n) // T):
                    segs.append(h_ref[j, pl.ds(TP * s, T), :])
                parts.append(jnp.concatenate(segs, axis=0))
            hcat = jnp.concatenate(parts, axis=1).astype(jnp.bfloat16)
            y = lax.dot_general(hcat, ccat_ref[...], _NT, preferred_element_type=jnp.float32)
            dn = jnp.dot(act[off:off + n], wd_ref[...], preferred_element_type=jnp.float32)
            start = c * LC + off if isinstance(c, int) else pl.multiple_of(c * LC + off, 128)
            x, xn = normalize(x_ref[pl.ds(start, n), :], st_ref[sl, 0, off:off + n, :],
                              st_ref[sl, 1, off:off + n, :])
            obuf[c, off:off + n, :] = (x + xn * a_ref[4:5, :]) + y + dn
            cpo(c, k).start()

    @pl.when(step == 0)
    def _first():
        cpx(0).start()
        cp(0).start()
        cpx(1).start()
        cp(1).start()
        lre = row(lre_r)
        lim = row(lim_r)
        dt = jnp.exp(row(ldt_r)).astype(jnp.bfloat16).astype(jnp.float32)
        mag = jnp.exp(dt * lre)
        ar = mag * jnp.cos(dt * lim)
        ai = mag * jnp.sin(dt * lim)
        nr = ar - 1.0
        ni = ai
        den = lre * lre + lim * lim
        cfr = 2.0 * ((nr * lre + ni * lim) / den)
        cfi = 2.0 * ((ni * lre - nr * lim) / den)
        a_ref[0:1, :] = ar
        a_ref[1:2, :] = ai
        pr, pi = ar, ai
        k = 1
        while k < T:
            pr, pi = _cmul(pr, pi, pr, pi)
            k *= 2
        a_ref[2:3, :] = pr
        a_ref[3:4, :] = pi
        a_ref[4:5, :] = row(dsk_ref)
        a_ref[5:8, :] = jnp.zeros((3, P), jnp.float32)
        carry_ref[...] = jnp.zeros((8, P), jnp.float32)

        cpx(0).wait()
        ma, ra = stats(x_ref[0:HC, :])
        ma, ra = bcast(ma), bcast(ra)
        st_ref[0, 0, 0:HC, :] = ma
        st_ref[0, 1, 0:HC, :] = ra
        xa = normalize(x_ref[0:HC, :], ma, ra)[1].astype(jnp.bfloat16)
        cp(0).wait()
        cpx(1).wait()
        cp(2).start()
        store_bu(lax.dot_general(xa, bre_ref[...], _NT, preferred_element_type=jnp.float32), 0, 0)
        mb, rb = stats(x_ref[HC:LC, :])
        mb, rb = bcast(mb), bcast(rb)
        st_ref[0, 0, HC:LC, :] = mb
        st_ref[0, 1, HC:LC, :] = rb
        xb = normalize(x_ref[HC:LC, :], mb, rb)[1].astype(jnp.bfloat16)
        store_bu(lax.dot_general(xb, bre_ref[...], _NT, preferred_element_type=jnp.float32), 0, S // 2)
        xnb = jnp.concatenate([xa, xb], axis=0)
        cp(1).wait()
        store_bu(lax.dot_general(xnb, bim_ref[...], _NT, preferred_element_type=jnp.float32), 4, 0)
        cp(2).wait()
        cp(3).start()
        cp(4).start()
        cp(5).start()
        g = lax.dot_general(xnb, wg_ref[...], _NT, preferred_element_type=jnp.float32)
        scan(0, 2)
        cp(3).wait()
        cp(6).start()
        for c in range(2, 2 * NC):
            cpx(c).start()
        u = lax.dot_general(xnb, wu_ref[...], _NT, preferred_element_type=jnp.float32)
        scan(2, 2)
        act = (jax.nn.gelu(g, approximate=True) * u).astype(jnp.bfloat16)
        cpx(2).wait()
        cpx(3).wait()
        cp(4).wait()
        cp(5).wait()
        cp(6).wait()
        ln_next(1, 1)
        c_re = cre_ref[...].astype(jnp.float32)
        c_im = cim_ref[...].astype(jnp.float32)
        ccat_ref[:, 0:P] = (c_re * cfr - c_im * cfi).astype(jnp.bfloat16)
        ccat_ref[:, P:2 * P] = (c_re * (-cfi) - c_im * cfr).astype(jnp.bfloat16)
        finish(act, 0, 0)
        for c in range(4, 2 * NC):
            cpx(c).wait()

    @pl.when(step > 0)
    def _rest():
        xnb = normalize(x_ref[rows(step, LC), :], st_ref[slot, 0], st_ref[slot, 1])[1].astype(jnp.bfloat16)
        store_bu(lax.dot_general(xnb, bre_ref[...], _NT, preferred_element_type=jnp.float32), 0, 0)
        store_bu(lax.dot_general(xnb, bim_ref[...], _NT, preferred_element_type=jnp.float32), 4, 0)
        g = lax.dot_general(xnb, wg_ref[...], _NT, preferred_element_type=jnp.float32)
        u = lax.dot_general(xnb, wu_ref[...], _NT, preferred_element_type=jnp.float32)
        act = (jax.nn.gelu(g, approximate=True) * u).astype(jnp.bfloat16)
        scan()
        ln_next(jnp.minimum(step + 1, NC - 1), 1 - slot)
        finish(act, step, slot)

        @pl.when(step == NC - 1)
        def _():
            for c in range(NC):
                for k in range(NP):
                    cpo(c, k).wait()


@jax.jit
def pallas_parallel_sum__ssm_conv_s5__geglu_ffn__prompt_kernel(
    A_x, A_Lambda_re, A_Lambda_im, A_B_re, A_B_im, A_C_re, A_C_im, A_log_dt, A_Dskip,
    B_x, B_w_gate, B_w_up, B_w_down,
):
    x2 = A_x.reshape(L, D)
    full = lambda shape: pl.BlockSpec(shape, lambda i: (0,) * len(shape))
    anyspec = pl.BlockSpec(memory_space=pl.ANY)
    out = pl.pallas_call(
        _kernel,
        grid=(NC,),
        in_specs=[
            full((P,)), full((P,)), full((P,)),
            full((D,)),
            anyspec, anyspec, anyspec, anyspec, anyspec, anyspec, anyspec, anyspec,
        ],
        out_specs=anyspec,
        out_shape=jax.ShapeDtypeStruct((L, D), jnp.float32),
        scratch_shapes=[
            pltpu.VMEM((L, D), jnp.bfloat16),
            pltpu.VMEM((P, D), jnp.bfloat16),
            pltpu.VMEM((P, D), jnp.bfloat16),
            pltpu.VMEM((D, P), jnp.bfloat16),
            pltpu.VMEM((D, P), jnp.bfloat16),
            pltpu.VMEM((F, D), jnp.bfloat16),
            pltpu.VMEM((F, D), jnp.bfloat16),
            pltpu.VMEM((F, D), jnp.bfloat16),
            pltpu.SemaphoreType.DMA((7,)),
            pltpu.SemaphoreType.DMA((2 * NC,)),
            pltpu.VMEM((D, 2 * P), jnp.bfloat16),
            pltpu.VMEM((8, P), jnp.float32),
            pltpu.VMEM((8, P), jnp.float32),
            pltpu.VMEM((8, S * TP, 128), jnp.float32),
            pltpu.VMEM((8, S * TP, 128), jnp.float32),
            pltpu.VMEM((2, 2, LC, 128), jnp.float32),
            pltpu.VMEM((NC, LC, D), jnp.float32),
            pltpu.SemaphoreType.DMA((NC * NP,)),
        ],
        compiler_params=pltpu.CompilerParams(
            dimension_semantics=("arbitrary",),
            vmem_limit_bytes=64 * 1024 * 1024,
        ),
    )(A_Lambda_re, A_Lambda_im, A_log_dt, A_Dskip,
      x2, A_B_re, A_B_im, A_C_re, A_C_im, B_w_gate.T, B_w_up.T, B_w_down)
    return out.reshape(1, L, D)
```
